```python
import jax
import jax.numpy as jnp

def _softmax(x, axis=-1):
    return jax.nn.softmax(x, axis=axis)
def _gelu(x):
    return jax.nn.gelu(x, approximate=True)
def _silu(x):
    return jax.nn.silu(x)
def _sigmoid(x):
    return jax.nn.sigmoid(x)
def _layernorm(x, axis=-1, eps=1e-5):
    m = jnp.mean(x, axis=axis, keepdims=True)
    v = jnp.var(x, axis=axis, keepdims=True)
    return (x - m) / jnp.sqrt(v + eps)
def _scatter_add(tgt, idx, src, axis=0):
    return tgt.at[idx].add(src)
def _segment_sum(src, seg, n):
    return jax.ops.segment_sum(src, seg, n)
class _Rng:
    def __init__(self, key):
        self._k = key
    def _next(self):
        self._k, sub = jax.random.split(self._k)
        return sub
    def normal(self, shape):
        return jax.random.normal(self._next(), shape, dtype=jnp.bfloat16)
    def randint(self, lo, hi, shape):
        return jax.random.randint(self._next(), shape, lo, hi, dtype=jnp.int32)
    def uniform(self, shape, lo=0.0, hi=1.0):
        return jax.random.uniform(self._next(), shape, jnp.bfloat16, lo, hi)
    def permutation(self, n):
        return jax.random.permutation(self._next(), n)


kernel_name = 'sequential_preLN__sliding_block_cached__glu_gated_swiglu__decode'

def setup_inputs():
    _rng = _Rng(jax.random.key(int.from_bytes(__import__("os").urandom(4), "little")))
    _w = (lambda a: (lambda t: t.astype(jnp.bfloat16) if jnp.issubdtype(t.dtype, jnp.floating) else t)(jnp.asarray(a)))
    def _A_setup():
        B, Sq, D = 1, 1, 640
        Hq, Hkv, Sk, Dh = 32, 32, 32768, 192
        assert Hq % Hkv == 0, (Hq, Hkv)
        return {
            "x": _w((lambda *s: _rng.normal(s) * 0.05)(B, Sq, D)),
            "k_cache": _w((lambda *s: _rng.normal(s) * 0.05)(B, Hkv, Sk, Dh)),
            "v_cache": _w((lambda *s: _rng.normal(s) * 0.05)(B, Hkv, Sk, Dh)),
            "wq": _w((lambda *s: _rng.normal(s) * 0.05)(D, Hq * Dh) * (D ** -0.5)),
            "wo": _w((lambda *s: _rng.normal(s) * 0.05)(Hq * Dh, D) * ((Hq * Dh) ** -0.5)),
        }
    _A_in = _A_setup()

    def _B_setup():
        B, S, D, F = 1, 1, 640, 1536
        return {
            "x": _w((lambda *s: _rng.normal(s) * 0.05)(B, S, D)),
            "w1": _w((lambda *s: _rng.normal(s) * 0.05)(D, F) * (2.0 / D) ** 0.5),
            "w3": _w((lambda *s: _rng.normal(s) * 0.05)(D, F) * (2.0 / D) ** 0.5),
            "w2": _w((lambda *s: _rng.normal(s) * 0.05)(F, D) * (2.0 / F) ** 0.5),
        }
    _B_in = _B_setup()

    return {
        "A_x": _A_in["x"],
        "A_k_cache": _A_in["k_cache"],
        "A_v_cache": _A_in["v_cache"],
        "A_wq": _A_in["wq"],
        "A_wo": _A_in["wo"],
        "B_x": _B_in["x"],
        "B_w1": _B_in["w1"],
        "B_w3": _B_in["w3"],
        "B_w2": _B_in["w2"],
    }

def reference(A_x, A_k_cache, A_v_cache, A_wq, A_wo, B_x, B_w1, B_w3, B_w2):
    def _A_ref(x, k_cache, v_cache, wq, wo):
        B, Sq, D = x.shape
        Hq, Dh = 32, 192
        Hkv, Sk = k_cache.shape[1], k_cache.shape[2]
        W = min(4096, max(256, Sk // 4))
        rep = Hq // Hkv
        q = (lambda x, *d: x.transpose(*d))((x @ wq).reshape(B, Sq, Hq, Dh), 0, 2, 1, 3)
        k = jnp.repeat(k_cache[:, :, Sk - W:, :], rep, axis=1)
        v = jnp.repeat(v_cache[:, :, Sk - W:, :], rep, axis=1)
        scores = jnp.einsum("bhqd,bhkd->bhqk", q, k) * (Dh ** -0.5)
        p = _softmax(scores, axis=-1)
        o = jnp.einsum("bhqk,bhkd->bhqd", p, v)
        return (lambda x, *d: x.transpose(*d))(o, 0, 2, 1, 3).reshape(B, Sq, Hq * Dh) @ wo

    def _B_ref(x, w1, w3, w2):
        gate = jnp.einsum("bsd,df->bsf", x, w1)
        up = jnp.einsum("bsd,df->bsf", x, w3)
        h = _silu(gate) * up
        out = jnp.einsum("bsf,fd->bsd", h, w2)
        return out

    x = A_x
    h = x + _A_ref(_layernorm(x, axis=-1), A_k_cache, A_v_cache, A_wq, A_wo)
    h2 = h + _B_ref(_layernorm(h, axis=-1), B_w1, B_w3, B_w2)
    return h2
```

```python
import functools
import jax
import jax.numpy as jnp
from jax.experimental import pallas as pl
from jax.experimental.pallas import tpu as pltpu

D = 640
HQ = 32
DH = 192
SK = 32768
WIN = 4096
F = 1536
PAIR = 2 * DH
NPAIR = HQ // 2
OFF = SK - WIN
EPS = 1e-5


def _layernorm(x):
    m = jnp.mean(x, axis=-1, keepdims=True)
    xc = x - m
    v = jnp.mean(xc * xc, axis=-1, keepdims=True)
    return xc / jnp.sqrt(v + EPS)


def make_kernel(NBUF=2, NCH=512, W2_SPLITS=(768, 1280, 1536), name="fused"):
    n_w2 = len(W2_SPLITS)

    def kernel(x_hbm, k_hbm, v_hbm, wq_hbm, wo_hbm, w1_hbm, w3_hbm, w2_hbm,
               o_ref,
               x_v, wq_v, wo_v, w1_v, w3_v, w2_v, k_buf, v_buf, q_blk,
               w_sems, k_sems, v_sems):
        def k_copy(p, slot):
            return pltpu.make_async_copy(
                k_hbm.at[pl.ds(p * PAIR, PAIR), pl.ds(OFF, WIN)], k_buf.at[slot], k_sems.at[slot])

        def v_copy(p, slot):
            return pltpu.make_async_copy(
                v_hbm.at[pl.ds(p * PAIR, PAIR), pl.ds(OFF, WIN)], v_buf.at[slot], v_sems.at[slot])

        x_cp = pltpu.make_async_copy(x_hbm, x_v, w_sems.at[0])
        wq_cp = pltpu.make_async_copy(wq_hbm, wq_v, w_sems.at[1])
        wo_cp = pltpu.make_async_copy(wo_hbm, wo_v, w_sems.at[2])
        w1_cp = pltpu.make_async_copy(w1_hbm, w1_v, w_sems.at[3])
        w3_cp = pltpu.make_async_copy(w3_hbm, w3_v, w_sems.at[4])
        w2_cps = []
        lo = 0
        for i, hi in enumerate(W2_SPLITS):
            w2_cps.append(pltpu.make_async_copy(w2_hbm.at[pl.ds(lo, hi - lo)], w2_v.at[pl.ds(lo, hi - lo)], w_sems.at[5 + i]))
            lo = hi

        wq_cp.start()
        x_cp.start()
        wo_cp.start()
        for p in range(NBUF):
            k_copy(p, p).start()
            v_copy(p, p).start()

        x_cp.wait()
        x8 = jnp.broadcast_to(x_v[...].astype(jnp.float32), (8, D))
        xn = _layernorm(x8).astype(jnp.bfloat16)
        row = jax.lax.broadcasted_iota(jnp.int32, (8, PAIR), 0)
        col = jax.lax.broadcasted_iota(jnp.int32, (8, PAIR), 1)
        diag = ((row == 0) & (col < DH)) | ((row == 1) & (col >= DH))
        wq_cp.wait()
        for p in range(NPAIR):
            qp = jnp.dot(xn, wq_v[:, p * PAIR:(p + 1) * PAIR], preferred_element_type=jnp.float32)
            q_blk[p] = jnp.where(diag, qp, 0.0).astype(jnp.bfloat16)

        wo_cp.wait()
        scale = DH ** -0.5

        def pair_body(p, acc):
            slot = p % NBUF
            qb = q_blk[p]
            k_copy(p, slot).wait()
            s_parts = []
            for c in range(WIN // NCH):
                kc = k_buf[slot, :, c * NCH:(c + 1) * NCH]
                s_parts.append(jnp.dot(qb, kc, preferred_element_type=jnp.float32))
            s = jnp.concatenate(s_parts, axis=1) * scale

            @pl.when(p + NBUF < NPAIR)
            def _():
                k_copy(p + NBUF, slot).start()

            m = jnp.max(s, axis=-1, keepdims=True)
            e = jnp.exp(s - m)
            l = jnp.sum(e, axis=-1, keepdims=True)
            eb = e.astype(jnp.bfloat16)
            v_copy(p, slot).wait()
            o = jnp.zeros((8, PAIR), jnp.float32)
            for c in range(WIN // NCH):
                vc = v_buf[slot, :, c * NCH:(c + 1) * NCH]
                o = o + jax.lax.dot_general(eb[:, c * NCH:(c + 1) * NCH], vc, (((1,), (1,)), ((), ())),
                                            preferred_element_type=jnp.float32)

            @pl.when(p + NBUF < NPAIR)
            def _():
                v_copy(p + NBUF, slot).start()

            @pl.when(p + NBUF == NPAIR - 1)
            def _():
                w1_cp.start()
                w3_cp.start()
                for c in w2_cps:
                    c.start()

            o = jnp.where(diag, o / l, 0.0).astype(jnp.bfloat16)
            wo_p = wo_v[pl.ds(pl.multiple_of(p * PAIR, PAIR), PAIR), :]
            return acc + jnp.dot(o, wo_p, preferred_element_type=jnp.float32)

        acc = jax.lax.fori_loop(0, NPAIR, pair_body, jnp.zeros((8, D), jnp.float32))

        attn = jnp.sum(acc, axis=0, keepdims=True)
        h = x8 + jnp.broadcast_to(attn, (8, D))
        hn = _layernorm(h).astype(jnp.bfloat16)
        w1_cp.wait()
        gate = jnp.dot(hn, w1_v[...], preferred_element_type=jnp.float32)
        w3_cp.wait()
        up = jnp.dot(hn, w3_v[...], preferred_element_type=jnp.float32)
        mid = (gate * jax.nn.sigmoid(gate) * up).astype(jnp.bfloat16)
        out = h
        lo = 0
        for i, hi in enumerate(W2_SPLITS):
            w2_cps[i].wait()
            out = out + jnp.dot(mid[:, lo:hi], w2_v[lo:hi, :], preferred_element_type=jnp.float32)
            lo = hi
        o_ref[...] = out[0:1, :].astype(o_ref.dtype)

    def f(A_x, A_k_cache, A_v_cache, A_wq, A_wo, B_x, B_w1, B_w3, B_w2):
        kT = jnp.transpose(A_k_cache, (0, 1, 3, 2)).reshape(HQ * DH, SK)
        vT = jnp.transpose(A_v_cache, (0, 1, 3, 2)).reshape(HQ * DH, SK)
        x2 = A_x.reshape(1, D)
        hbm = pl.BlockSpec(memory_space=pltpu.HBM)
        out = pl.pallas_call(
            kernel,
            out_shape=jax.ShapeDtypeStruct((1, D), jnp.bfloat16),
            in_specs=[hbm] * 8,
            out_specs=pl.BlockSpec(memory_space=pltpu.VMEM),
            scratch_shapes=[
                pltpu.VMEM((1, D), jnp.bfloat16),
                pltpu.VMEM((D, HQ * DH), jnp.bfloat16),
                pltpu.VMEM((HQ * DH, D), jnp.bfloat16),
                pltpu.VMEM((D, F), jnp.bfloat16),
                pltpu.VMEM((D, F), jnp.bfloat16),
                pltpu.VMEM((F, D), jnp.bfloat16),
                pltpu.VMEM((NBUF, PAIR, WIN), jnp.bfloat16),
                pltpu.VMEM((NBUF, PAIR, WIN), jnp.bfloat16),
                pltpu.VMEM((NPAIR, 8, PAIR), jnp.bfloat16),
                pltpu.SemaphoreType.DMA((5 + n_w2,)),
                pltpu.SemaphoreType.DMA((NBUF,)),
                pltpu.SemaphoreType.DMA((NBUF,)),
            ],
            compiler_params=pltpu.CompilerParams(vmem_limit_bytes=96 * 1024 * 1024),
            name=name,
        )(x2, kT, vT, A_wq, A_wo, B_w1, B_w3, B_w2)
        return out.reshape(1, 1, D)

    return f


_impl = make_kernel(NBUF=2, NCH=512, name="fused_decode_block")


@jax.jit
def pallas_sequential_preLN__sliding_block_cached__glu_gated_swiglu__decode_kernel(
    A_x: jax.Array,
    A_k_cache: jax.Array,
    A_v_cache: jax.Array,
    A_wq: jax.Array,
    A_wo: jax.Array,
    B_x: jax.Array,
    B_w1: jax.Array,
    B_w3: jax.Array,
    B_w2: jax.Array,
):
    return _impl(A_x, A_k_cache, A_v_cache, A_wq, A_wo, B_x, B_w1, B_w3, B_w2)
```

```python
import jax
import jax.numpy as jnp
from jax.experimental import pallas as pl
from jax.experimental.pallas import tpu as pltpu

D = 640
HQ = 32
DH = 192
SK = 32768
WIN = 4096
F = 1536
PAIR = 2 * DH
NPAIR = HQ // 2
OFF = SK - WIN
EPS = 1e-5
NT = (((1,), (1,)), ((), ()))
SC = 512
NSL = WIN // SC


def _layernorm(x):
    m = jnp.mean(x, axis=-1, keepdims=True)
    xc = x - m
    v = jnp.mean(xc * xc, axis=-1, keepdims=True)
    return xc / jnp.sqrt(v + EPS)


class Unit:
    def __init__(self, lo, hi, whole, nbytes):
        self.lo, self.hi, self.whole, self.nbytes = lo, hi, whole, nbytes

    def start(self):
        self.lo().start(priority=1)
        self.hi().start(priority=0)

    def wait(self):
        self.whole().wait()


class Pump:
    def __init__(self, units, limit, started=0):
        self.units, self.limit = units, limit
        self.n_started, self.n_waited = started, 0
        self.inflight = sum(u.nbytes for u in units[:started])

    def fill(self):
        while self.n_started < len(self.units) and self.inflight + self.units[self.n_started].nbytes <= self.limit:
            u = self.units[self.n_started]
            u.start()
            self.inflight += u.nbytes
            self.n_started += 1

    def step(self):
        u = self.units[self.n_waited]
        assert self.n_waited < self.n_started
        u.wait()
        self.inflight -= u.nbytes
        self.n_waited += 1
        self.fill()

    def run(self, n, pieces=()):
        done = 0
        for i in range(n):
            self.step()
            want = ((i + 1) * len(pieces)) // n
            while done < want:
                pieces[done]()
                done += 1


def make_kernel(U=8, name="fused3", do_compute=True, nochecks=False,
                WQ_G=8, WO_G=16, WO_SPLIT=(0, 6, 11, 16), W1_G=4, W1_C=512,
                W2_PIECES=((384, 48), (384, 48), (384, 48), (256, 32), (128, 32)), LIMIT=None, NS=4, KAHEAD=2, PRO_K=None):
    UR = PAIR // U
    KV_UNIT_BYTES = UR * SC * 2
    limit = LIMIT or KAHEAD * U * KV_UNIT_BYTES

    def kernel(x_hbm, k_hbm, v_hbm, wq_hbm, wo_hbm, w1_hbm, w3_hbm, w2_hbm,
               o_ref,
               x_v, wq_v, wo_v, w1_v, w3_v, w2_v, kv_buf, q_blk, s_ref,
               w_sems, kv_sems):

        def group_unit(src, dst, sem, g0, g1, r0, nr, c0, nc):
            def cp(a, b):
                return lambda: pltpu.make_async_copy(
                    src.at[pl.ds(a, b - a), pl.ds(r0, nr), pl.ds(c0, nc)],
                    dst.at[pl.ds(a, b - a), pl.ds(r0, nr), pl.ds(c0, nc)], sem)
            return Unit(cp(g0, g1 - 1), cp(g1 - 1, g1), cp(g0, g1), (g1 - g0) * nr * nc * 2)

        def row_unit(src, dst, sem, r0, nr, hi):
            def cp(a, b):
                return lambda: pltpu.make_async_copy(src.at[pl.ds(r0 + a, b - a)], dst.at[pl.ds(r0 + a, b - a)], sem)
            return Unit(cp(0, nr - hi), cp(nr - hi, nr), cp(0, nr), nr * src.shape[-1] * 2)

        def kv_slice_units(g, p):
            if g >= 2 * NSL:
                g, p = g - 2 * NSL, p + 1
            src = k_hbm if g < NSL else v_hbm
            c0 = OFF + (g % NSL) * SC
            slot = g % NS

            def cp(u, a, b):
                return lambda: pltpu.make_async_copy(
                    src.at[pl.ds(p * PAIR + u * UR + a, b - a), pl.ds(c0, SC)],
                    kv_buf.at[slot, pl.ds(u * UR + a, b - a)], kv_sems.at[slot])
            return [Unit(cp(u, 0, UR - 8), cp(u, UR - 8, UR), cp(u, 0, UR), KV_UNIT_BYTES) for u in range(U)]

        wq_units = [group_unit(wq_hbm, wq_v, w_sems.at[1], 0, WQ_G, 8 * j, 8, c * SC, SC)
                    for j in range(D // WQ_G // 8) for c in range(HQ * DH // SC)]
        wo_units = [group_unit(wo_hbm, wo_v, w_sems.at[2], WO_SPLIT[s], WO_SPLIT[s + 1], 8 * j, 8, 0, D)
                    for j in range(HQ * DH // WO_G // 8) for s in range(len(WO_SPLIT) - 1)]
        w1_units = [group_unit(w1_hbm, w1_v, w_sems.at[3], 0, W1_G, 8 * j, 8, c * W1_C, W1_C)
                    for j in range(D // W1_G // 8) for c in range(F // W1_C)]
        w3_units = [group_unit(w3_hbm, w3_v, w_sems.at[4], 0, W1_G, 8 * j, 8, c * W1_C, W1_C)
                    for j in range(D // W1_G // 8) for c in range(F // W1_C)]
        w2_groups, lo = [], 0
        for i, (rows, ur) in enumerate(W2_PIECES):
            w2_groups.append((lo, lo + rows, [row_unit(w2_hbm, w2_v, w_sems.at[5 + i], lo + ur * j, ur, 8)
                                              for j in range(rows // ur)]))
            lo += rows
        w2_units = [u for g in w2_groups for u in g[2]]
        x_cp = pltpu.make_async_copy(x_hbm, x_v, w_sems.at[0])

        x_cp.start()
        pro = Pump(wq_units + wo_units + [u for g in range(KAHEAD) for u in kv_slice_units(g, 0)], limit)
        pro.fill()
        pro.run(8)
        x_cp.wait()
        x8 = jnp.broadcast_to(x_v[...].astype(jnp.float32), (8, D))
        xn = _layernorm(x8).astype(jnp.bfloat16)
        pro.run(len(wq_units) - 8)

        row = jax.lax.broadcasted_iota(jnp.int32, (8, PAIR), 0)
        col = jax.lax.broadcasted_iota(jnp.int32, (8, PAIR), 1)
        diag = ((row == 0) & (col < DH)) | ((row == 1) & (col >= DH))

        def q_piece(j):
            def f():
                if not do_compute:
                    return
                w = wq_v[:, :, j * PAIR:(j + 1) * PAIR].reshape(D, PAIR)
                qp = jnp.dot(xn, w, preferred_element_type=jnp.float32)
                q_blk[j] = jnp.where(diag, qp, 0.0).astype(jnp.bfloat16)
            return f

        pro.run(len(wo_units), [q_piece(j) for j in range(NPAIR)])
        assert pro.n_started == len(pro.units)
        scale = DH ** -0.5

        def qk_piece(p, i, t):
            if not do_compute:
                return
            s = jnp.dot(q_blk[p], kv_buf[i % NS], preferred_element_type=jnp.float32) * scale
            s_ref[:, i * SC:(i + 1) * SC] = s
            for c in range(SC // 128):
                sc = s[:, c * 128:(c + 1) * 128]
                t["mx"] = sc if "mx" not in t else jnp.maximum(t["mx"], sc)

        def pv_piece(p, i, t):
            if not do_compute:
                return
            if i == 0:
                t["m"] = jnp.max(t["mx"], axis=-1, keepdims=True)
            e = jnp.exp(s_ref[:, i * SC:(i + 1) * SC] - t["m"])
            for c in range(SC // 128):
                ec = e[:, c * 128:(c + 1) * 128]
                t["l"] = ec if "l" not in t else t["l"] + ec
            o = jax.lax.dot_general(e.astype(jnp.bfloat16), kv_buf[(NSL + i) % NS], NT,
                                    preferred_element_type=jnp.float32)
            t["o"] = o if "o" not in t else t["o"] + o

        def finalize(p, t, acc):
            if not do_compute:
                return acc
            l = jnp.sum(t["l"], axis=-1, keepdims=True)
            o = jnp.where(diag, t["o"] / l, 0.0).astype(jnp.bfloat16)
            if WO_G == NPAIR:
                w = wo_v[p]
            else:
                per = NPAIR // WO_G
                r0 = (p % per) * PAIR
                if not isinstance(p, int):
                    r0 = pl.multiple_of(r0, PAIR)
                w = wo_v[p // per, pl.ds(r0, PAIR), :]
            return acc + jnp.dot(o, w, preferred_element_type=jnp.float32)

        def slice_compute(p, g, t):
            if g < NSL:
                qk_piece(p, g, t)
            else:
                pv_piece(p, g - NSL, t)

        def pair_body(p, acc):
            t = {}
            for g in range(2 * NSL):
                cur, nxt = kv_slice_units(g, p), kv_slice_units(g + KAHEAD, p)
                for u in range(U):
                    cur[u].wait()
                    nxt[u].start()
                slice_compute(p, g, t)
            return finalize(p, t, acc)

        acc = jax.lax.fori_loop(0, NPAIR - 1, pair_body, jnp.zeros((8, D), jnp.float32))

        pl_ = NPAIR - 1
        t = {}
        kv_last = [u for g in range(2 * NSL) for u in kv_slice_units(g, pl_)]
        epi = Pump(kv_last + w1_units + w3_units + w2_units, limit, started=KAHEAD * U)
        for g in range(2 * NSL):
            epi.run(U)
            slice_compute(pl_, g, t)
        acc = finalize(pl_, t, acc)

        attn = jnp.sum(acc, axis=0, keepdims=True)
        h = x8 + jnp.broadcast_to(attn, (8, D))
        hn = _layernorm(h).astype(jnp.bfloat16)
        NG = 6
        GC = F // NG
        gate, mid = [None] * NG, [None] * NG

        def gate_piece(i):
            def f():
                if do_compute:
                    w = w1_v[:, :, i * GC:(i + 1) * GC].reshape(D, GC)
                    gate[i] = jnp.dot(hn, w, preferred_element_type=jnp.float32)
            return f

        def up_piece(i):
            def f():
                if do_compute:
                    w = w3_v[:, :, i * GC:(i + 1) * GC].reshape(D, GC)
                    up = jnp.dot(hn, w, preferred_element_type=jnp.float32)
                    mid[i] = (gate[i] * jax.nn.sigmoid(gate[i]) * up).astype(jnp.bfloat16)
            return f

        epi.run(len(w1_units))
        epi.run(len(w3_units), [gate_piece(i) for i in range(NG)])
        out = h
        for gi, (lo, hi, units) in enumerate(w2_groups):
            epi.run(len(units), [up_piece(i) for i in range(NG)] if gi == 0 else ())
            if do_compute:
                if gi == 0:
                    midc = jnp.concatenate(mid, axis=1)
                out = out + jnp.dot(midc[:, lo:hi], w2_v[lo:hi, :], preferred_element_type=jnp.float32)
        o_ref[...] = out[0:1, :].astype(o_ref.dtype)

    def f(A_x, A_k_cache, A_v_cache, A_wq, A_wo, B_x, B_w1, B_w3, B_w2):
        kT = jnp.transpose(A_k_cache, (0, 1, 3, 2)).reshape(HQ * DH, SK)
        vT = jnp.transpose(A_v_cache, (0, 1, 3, 2)).reshape(HQ * DH, SK)
        x2 = A_x.reshape(1, D)
        wq3 = A_wq.reshape(WQ_G, D // WQ_G, HQ * DH)
        wo3 = A_wo.reshape(WO_G, HQ * DH // WO_G, D)
        w13 = B_w1.reshape(W1_G, D // W1_G, F)
        w33 = B_w3.reshape(W1_G, D // W1_G, F)
        hbm = pl.BlockSpec(memory_space=pltpu.HBM)
        out = pl.pallas_call(
            kernel,
            out_shape=jax.ShapeDtypeStruct((1, D), jnp.bfloat16),
            in_specs=[hbm] * 8,
            out_specs=pl.BlockSpec(memory_space=pltpu.VMEM),
            scratch_shapes=[
                pltpu.VMEM((1, D), jnp.bfloat16),
                pltpu.VMEM(wq3.shape, jnp.bfloat16),
                pltpu.VMEM(wo3.shape, jnp.bfloat16),
                pltpu.VMEM(w13.shape, jnp.bfloat16),
                pltpu.VMEM(w33.shape, jnp.bfloat16),
                pltpu.VMEM((F, D), jnp.bfloat16),
                pltpu.VMEM((NS, PAIR, SC), jnp.bfloat16),
                pltpu.VMEM((NPAIR, 8, PAIR), jnp.bfloat16),
                pltpu.VMEM((8, WIN), jnp.float32),
                pltpu.SemaphoreType.DMA((5 + len(W2_PIECES),)),
                pltpu.SemaphoreType.DMA((NS,)),
            ],
            compiler_params=pltpu.CompilerParams(vmem_limit_bytes=64 * 1024 * 1024, disable_bounds_checks=nochecks),
            name=name,
        )(x2, kT, vT, wq3, wo3, w13, w33, B_w2)
        return out.reshape(1, 1, D)

    return f


_impl = make_kernel(U=8, KAHEAD=3, NS=4, name="fused_decode_block")


@jax.jit
def pallas_sequential_preLN__sliding_block_cached__glu_gated_swiglu__decode_kernel(
    A_x: jax.Array,
    A_k_cache: jax.Array,
    A_v_cache: jax.Array,
    A_wq: jax.Array,
    A_wo: jax.Array,
    B_x: jax.Array,
    B_w1: jax.Array,
    B_w3: jax.Array,
    B_w2: jax.Array,
):
    return _impl(A_x, A_k_cache, A_v_cache, A_wq, A_wo, B_x, B_w1, B_w3, B_w2)
```

```python
import jax
import jax.numpy as jnp
from jax.experimental import pallas as pl
from jax.experimental.pallas import tpu as pltpu

D = 640
HQ = 32
DH = 192
SK = 32768
WIN = min(4096, max(256, SK // 4))
F = 1536
EPS = 1e-5

PAIR = 2 * DH
NPAIR = HQ // 2
OFF = SK - WIN
SC = 512
NSL = WIN // SC
NS = 4
U = 8
UR = PAIR // U
KV_UNIT_BYTES = UR * SC * 2
NLO = 24
MHI = 16
IN_FLIGHT = NLO * KV_UNIT_BYTES
assert U <= MHI <= NLO <= (NS - 1) * U

WQ_G = 8
WO_SPLIT = (0, 6, 11, 16)
W13_G = 4
W2_PIECES = ((768, 48), (384, 48), (256, 32), (128, 32))
WQ_PER, WO_PER, W13_PER, W2_PER = 8, 12, 12, 8
NG = 6
NT = (((1,), (1,)), ((), ()))


def _layernorm(x):
    m = jnp.mean(x, axis=-1, keepdims=True)
    xc = x - m
    v = jnp.mean(xc * xc, axis=-1, keepdims=True)
    return xc / jnp.sqrt(v + EPS)


class Unit:
    def __init__(self, lo, hi, nbytes, group, sem_id):
        self.lo, self.hi, self.nbytes = lo, hi, nbytes
        self.group, self.sem_id = group, sem_id


class Pump:
    def __init__(self, units, lo_started=0, hi_started=0):
        self.units = units
        self.n_lo, self.n_hi, self.n_waited = lo_started, hi_started, 0
        self.inflight = sum(u.nbytes for u in units[:lo_started])
        self.left, self.last = {}, {}
        for i, u in enumerate(units):
            self.left[u.group] = self.left.get(u.group, 0) + 1
            self.last[u.group] = i
        self.owner = {}
        for u in units[:lo_started]:
            self.claim(u.sem_id, u.group)

    def claim(self, sem_id, group):
        prev = self.owner.get(sem_id)
        assert prev is None or prev == group or self.left[prev] == 0, ("semaphore in use", sem_id, prev, group)
        self.owner[sem_id] = group

    def fill(self):
        while self.n_lo < len(self.units) and self.inflight + self.units[self.n_lo].nbytes <= IN_FLIGHT:
            u = self.units[self.n_lo]
            self.claim(u.sem_id, u.group)
            u.lo().start(priority=1)
            self.inflight += u.nbytes
            self.n_lo += 1
        while self.n_hi < min(self.n_lo, self.n_waited + MHI):
            self.units[self.n_hi].hi().start(priority=0)
            self.n_hi += 1

    def step(self):
        u = self.units[self.n_waited]
        assert self.last[u.group] < self.n_hi <= self.n_lo, ("group not fully started", u.group)
        u.hi().wait()
        u.lo().wait()
        self.left[u.group] -= 1
        self.inflight -= u.nbytes
        self.n_waited += 1
        self.fill()

    def wait_units(self, n, pieces=()):
        done = 0
        for i in range(n):
            self.step()
            while done < ((i + 1) * len(pieces)) // n:
                pieces[done]()
                done += 1

    def landed(self, units):
        assert all(self.left[u.group] == 0 for u in units)


class GroupLabels:
    def __init__(self, first_sem):
        self.count, self.first_sem = -1, first_sem

    def label(self, tag, i, per):
        if i % per == 0:
            self.count += 1
        return (tag, i // per), (self.first_sem + self.count) % NS


def _kernel(x_hbm, k_hbm, v_hbm, wq_hbm, wo_hbm, w1_hbm, w3_hbm, w2_hbm,
            o_ref,
            x_v, wq_v, wo_v, w1_v, w3_v, w2_v, kv_buf, q_blk, s_ref, sems):

    def view_unit(src, dst, group, s, g0, g1, r0, c0, nc):
        def cp(a, b):
            return lambda: pltpu.make_async_copy(
                src.at[pl.ds(a, b - a), pl.ds(r0, 8), pl.ds(c0, nc)],
                dst.at[pl.ds(a, b - a), pl.ds(r0, 8), pl.ds(c0, nc)], sems.at[s])
        return Unit(cp(g0, g1 - 1), cp(g1 - 1, g1), (g1 - g0) * 8 * nc * 2, group, s)

    def row_unit(src, dst, group, s, r0, nr):
        def cp(a, b):
            return lambda: pltpu.make_async_copy(
                src.at[pl.ds(r0 + a, b - a)], dst.at[pl.ds(r0 + a, b - a)], sems.at[s])
        return Unit(cp(0, nr - 8), cp(nr - 8, nr), nr * src.shape[-1] * 2, group, s)

    def kv_units(g, p):
        group = ("kv", g)
        if g >= 2 * NSL:
            g, p = g - 2 * NSL, p + 1
        src = k_hbm if g < NSL else v_hbm
        c0 = OFF + (g % NSL) * SC
        slot = g % NS

        def cp(u, a, b):
            return lambda: pltpu.make_async_copy(
                src.at[pl.ds(p * PAIR + u * UR + a, b - a), pl.ds(c0, SC)],
                kv_buf.at[slot, pl.ds(u * UR + a, b - a)], sems.at[slot])
        return [Unit(cp(u, 0, UR - 8), cp(u, UR - 8, UR), KV_UNIT_BYTES, group, slot) for u in range(U)]

    n_wq = (D // WQ_G // 8) * (HQ * DH // SC)
    n_wo = (PAIR // 8) * (len(WO_SPLIT) - 1)
    labels = GroupLabels((-(-(-n_wq // WQ_PER) + -(-n_wo // WO_PER))) % NS)
    x_sem = (labels.first_sem - 1) % NS
    wq_units, wo_units = [], []
    for j in range(D // WQ_G // 8):
        for c in range(HQ * DH // SC):
            grp, s = labels.label("wq", len(wq_units), WQ_PER)
            wq_units.append(view_unit(wq_hbm, wq_v, grp, s, 0, WQ_G, 8 * j, c * SC, SC))
    for j in range(PAIR // 8):
        for k in range(len(WO_SPLIT) - 1):
            grp, s = labels.label("wo", len(wo_units), WO_PER)
            wo_units.append(view_unit(wo_hbm, wo_v, grp, s, WO_SPLIT[k], WO_SPLIT[k + 1], 8 * j, 0, D))
    labels = GroupLabels(0)
    w1_units, w3_units, w2_pieces = [], [], []
    for units, src, dst, tag in ((w1_units, w1_hbm, w1_v, "w1"), (w3_units, w3_hbm, w3_v, "w3")):
        for j in range(D // W13_G // 8):
            for c in range(F // SC):
                grp, s = labels.label(tag, len(units), W13_PER)
                units.append(view_unit(src, dst, grp, s, 0, W13_G, 8 * j, c * SC, SC))
    lo = 0
    for i, (rows, ur) in enumerate(W2_PIECES):
        units = []
        for j in range(rows // ur):
            grp, s = labels.label(("w2", i), j, W2_PER)
            units.append(row_unit(w2_hbm, w2_v, grp, s, lo + ur * j, ur))
        w2_pieces.append((lo, lo + rows, units))
        lo += rows
    assert lo == F

    x_cp = pltpu.make_async_copy(x_hbm, x_v, sems.at[x_sem])
    first_kv = [u for g in range(NS - 1) for u in kv_units(g, 0)][:NLO]
    pro = Pump(wq_units + wo_units + first_kv)
    x_cp.start()
    pro.left["x"] = 1
    pro.claim(x_sem, "x")
    pro.fill()
    pro.wait_units(2)
    x_cp.wait()
    pro.left["x"] = 0
    x8 = jnp.broadcast_to(x_v[...].astype(jnp.float32), (8, D))
    xn = _layernorm(x8).astype(jnp.bfloat16)
    pro.wait_units(len(wq_units) - 2)
    pro.landed(wq_units)

    row = jax.lax.broadcasted_iota(jnp.int32, (8, PAIR), 0)
    col = jax.lax.broadcasted_iota(jnp.int32, (8, PAIR), 1)
    diag = ((row == 0) & (col < DH)) | ((row == 1) & (col >= DH))

    def q_piece(j):
        def f():
            w = wq_v[:, :, j * PAIR:(j + 1) * PAIR].reshape(D, PAIR)
            qp = jnp.dot(xn, w, preferred_element_type=jnp.float32)
            q_blk[j] = jnp.where(diag, qp, 0.0).astype(jnp.bfloat16)
        return f

    pro.wait_units(len(wo_units), [q_piece(j) for j in range(NPAIR)])
    pro.landed(wo_units)
    n_pro = len(wq_units) + len(wo_units)
    assert (pro.n_lo, pro.n_hi, pro.n_waited) == (n_pro + NLO, n_pro + MHI, n_pro)

    scale = DH ** -0.5

    def qk_piece(p, i, t):
        s = jnp.dot(q_blk[p], kv_buf[i % NS], preferred_element_type=jnp.float32) * scale
        s_ref[:, i * SC:(i + 1) * SC] = s
        for c in range(SC // 128):
            sc = s[:, c * 128:(c + 1) * 128]
            t["mx"] = sc if "mx" not in t else jnp.maximum(t["mx"], sc)

    def pv_piece(i, t):
        if i == 0:
            t["m"] = jnp.max(t["mx"], axis=-1, keepdims=True)
        e = jnp.exp(s_ref[:, i * SC:(i + 1) * SC] - t["m"])
        for c in range(SC // 128):
            ec = e[:, c * 128:(c + 1) * 128]
            t["l"] = ec if "l" not in t else t["l"] + ec
        o = jax.lax.dot_general(e.astype(jnp.bfloat16), kv_buf[(NSL + i) % NS], NT,
                                preferred_element_type=jnp.float32)
        t["o"] = o if "o" not in t else t["o"] + o

    def slice_compute(p, g, t):
        if g < NSL:
            qk_piece(p, g, t)
        else:
            pv_piece(g - NSL, t)

    def finalize(p, t, acc):
        l = jnp.sum(t["l"], axis=-1, keepdims=True)
        o = jnp.where(diag, t["o"] / l, 0.0).astype(jnp.bfloat16)
        return acc + jnp.dot(o, wo_v[p], preferred_element_type=jnp.float32)

    def pair_body(p, acc):
        t = {}
        for g in range(2 * NSL):
            cur = kv_units(g, p)
            for u in range(U):
                cur[u].hi().wait()
                cur[u].lo().wait()
                il, ih = g * U + u + NLO, g * U + u + MHI
                kv_units(il // U, p)[il % U].lo().start(priority=1)
                kv_units(ih // U, p)[ih % U].hi().start(priority=0)
            slice_compute(p, g, t)
        return finalize(p, t, acc)

    acc = jax.lax.fori_loop(0, NPAIR - 1, pair_body, jnp.zeros((8, D), jnp.float32))

    last = NPAIR - 1
    kv_last = [kv_units(g, last) for g in range(2 * NSL)]
    epi = Pump([u for us in kv_last for u in us] + w1_units + w3_units
               + [u for piece in w2_pieces for u in piece[2]], lo_started=NLO, hi_started=MHI)
    t = {}
    for g in range(2 * NSL):
        epi.wait_units(U)
        epi.landed(kv_last[g])
        slice_compute(last, g, t)
    acc = finalize(last, t, acc)

    attn = jnp.sum(acc, axis=0, keepdims=True)
    h = x8 + jnp.broadcast_to(attn, (8, D))
    hn = _layernorm(h).astype(jnp.bfloat16)
    gc = F // NG
    gate, mid = [None] * NG, [None] * NG

    def gate_piece(i):
        def f():
            w = w1_v[:, :, i * gc:(i + 1) * gc].reshape(D, gc)
            gate[i] = jnp.dot(hn, w, preferred_element_type=jnp.float32)
        return f

    def up_piece(i):
        def f():
            w = w3_v[:, :, i * gc:(i + 1) * gc].reshape(D, gc)
            up = jnp.dot(hn, w, preferred_element_type=jnp.float32)
            mid[i] = (gate[i] * jax.nn.sigmoid(gate[i]) * up).astype(jnp.bfloat16)
        return f

    epi.wait_units(len(w1_units))
    epi.landed(w1_units)
    epi.wait_units(len(w3_units), [gate_piece(i) for i in range(NG)])
    epi.landed(w3_units)
    out = h
    for i, (lo, hi, units) in enumerate(w2_pieces):
        epi.wait_units(len(units), [up_piece(c) for c in range(NG)] if i == 0 else ())
        epi.landed(units)
        if i == 0:
            midc = jnp.concatenate(mid, axis=1)
        out = out + jnp.dot(midc[:, lo:hi], w2_v[lo:hi, :], preferred_element_type=jnp.float32)
    assert epi.n_waited == len(epi.units)
    o_ref[...] = out[0:1, :].astype(o_ref.dtype)


@jax.jit
def pallas_sequential_preLN__sliding_block_cached__glu_gated_swiglu__decode_kernel(
    A_x: jax.Array,
    A_k_cache: jax.Array,
    A_v_cache: jax.Array,
    A_wq: jax.Array,
    A_wo: jax.Array,
    B_x: jax.Array,
    B_w1: jax.Array,
    B_w3: jax.Array,
    B_w2: jax.Array,
):
    del B_x
    assert A_x.shape == (1, 1, D) and A_k_cache.shape == A_v_cache.shape == (1, HQ, SK, DH)
    hbm = pl.BlockSpec(memory_space=pltpu.HBM)
    out = pl.pallas_call(
        _kernel,
        out_shape=jax.ShapeDtypeStruct((1, D), A_x.dtype),
        in_specs=[hbm] * 8,
        out_specs=pl.BlockSpec(memory_space=pltpu.VMEM),
        scratch_shapes=[
            pltpu.VMEM((1, D), jnp.bfloat16),
            pltpu.VMEM((WQ_G, D // WQ_G, HQ * DH), jnp.bfloat16),
            pltpu.VMEM((NPAIR, PAIR, D), jnp.bfloat16),
            pltpu.VMEM((W13_G, D // W13_G, F), jnp.bfloat16),
            pltpu.VMEM((W13_G, D // W13_G, F), jnp.bfloat16),
            pltpu.VMEM((F, D), jnp.bfloat16),
            pltpu.VMEM((NS, PAIR, SC), jnp.bfloat16),
            pltpu.VMEM((NPAIR, 8, PAIR), jnp.bfloat16),
            pltpu.VMEM((8, WIN), jnp.float32),
            pltpu.SemaphoreType.DMA((NS,)),
        ],
        compiler_params=pltpu.CompilerParams(vmem_limit_bytes=64 * 1024 * 1024),
        name="fused_decode_block",
    )(
        A_x.reshape(1, D),
        jnp.transpose(A_k_cache, (0, 1, 3, 2)).reshape(HQ * DH, SK),
        jnp.transpose(A_v_cache, (0, 1, 3, 2)).reshape(HQ * DH, SK),
        A_wq.reshape(WQ_G, D // WQ_G, HQ * DH),
        A_wo.reshape(NPAIR, PAIR, D),
        B_w1.reshape(W13_G, D // W13_G, F),
        B_w3.reshape(W13_G, D // W13_G, F),
        B_w2,
    )
    return out.reshape(1, 1, D)
```

```python
import jax
import jax.numpy as jnp
from jax.experimental import pallas as pl
from jax.experimental.pallas import tpu as pltpu

D = 640
HQ = 32
DH = 192
SK = 32768
WIN = min(4096, max(256, SK // 4))
F = 1536
EPS = 1e-5

PAIR = 2 * DH
NPAIR = HQ // 2
OFF = SK - WIN
SC = 512
NSL = WIN // SC
NS = 4
U = 8
UR = PAIR // U
KV_UNIT_BYTES = UR * SC * 2
NLO = 24
MHI = 16
IN_FLIGHT = NLO * KV_UNIT_BYTES
assert U <= MHI <= NLO <= (NS - 1) * U

WQ_G = 8
WO_SPLIT = (0, 6, 11, 16)
W13_G = 4
W2_PIECES = ((768, 48), (384, 48), (256, 32), (128, 32))
WQ_PER, WO_PER, W13_PER, W2_PER = 8, 12, 12, 8
NG = 6
NT = (((1,), (1,)), ((), ()))


def _layernorm(x):
    m = jnp.mean(x, axis=-1, keepdims=True)
    xc = x - m
    v = jnp.mean(xc * xc, axis=-1, keepdims=True)
    return xc / jnp.sqrt(v + EPS)


class Unit:
    def __init__(self, lo, hi, nbytes, group, sem_id):
        self.lo, self.hi, self.nbytes = lo, hi, nbytes
        self.group, self.sem_id = group, sem_id


class Pump:
    def __init__(self, units, lo_started=0, hi_started=0):
        self.units = units
        self.n_lo, self.n_hi, self.n_waited = lo_started, hi_started, 0
        self.inflight = sum(u.nbytes for u in units[:lo_started])
        self.left, self.last = {}, {}
        for i, u in enumerate(units):
            self.left[u.group] = self.left.get(u.group, 0) + 1
            self.last[u.group] = i
        self.owner = {}
        for u in units[:lo_started]:
            self.claim(u.sem_id, u.group)

    def claim(self, sem_id, group):
        prev = self.owner.get(sem_id)
        assert prev is None or prev == group or self.left[prev] == 0, ("semaphore in use", sem_id, prev, group)
        self.owner[sem_id] = group

    def fill(self):
        while self.n_lo < len(self.units) and self.inflight + self.units[self.n_lo].nbytes <= IN_FLIGHT:
            u = self.units[self.n_lo]
            self.claim(u.sem_id, u.group)
            u.lo().start(priority=1)
            self.inflight += u.nbytes
            self.n_lo += 1
        while self.n_hi < min(self.n_lo, self.n_waited + MHI):
            self.units[self.n_hi].hi().start(priority=0)
            self.n_hi += 1

    def step(self):
        u = self.units[self.n_waited]
        assert self.last[u.group] < self.n_hi <= self.n_lo, ("group not fully started", u.group)
        u.hi().wait()
        u.lo().wait()
        self.left[u.group] -= 1
        self.inflight -= u.nbytes
        self.n_waited += 1
        self.fill()

    def wait_units(self, n, pieces=()):
        done = 0
        for i in range(n):
            self.step()
            while done < ((i + 1) * len(pieces)) // n:
                pieces[done]()
                done += 1

    def landed(self, units):
        assert all(self.left[u.group] == 0 for u in units)


class GroupLabels:
    def __init__(self, first_sem):
        self.count, self.first_sem = -1, first_sem

    def label(self, tag, i, per):
        if i % per == 0:
            self.count += 1
        return (tag, i // per), (self.first_sem + self.count) % NS


def _kernel(x_hbm, k_hbm, v_hbm, wq_hbm, wo_hbm, w1_hbm, w3_hbm, w2_hbm,
            o_ref,
            x_v, wq_v, wo_v, w1_v, w3_v, w2_v, kv_buf, q_blk, s_ref, sems):

    def view_unit(src, dst, group, s, g0, g1, r0, c0, nc):
        def cp(a, b):
            return lambda: pltpu.make_async_copy(
                src.at[pl.ds(a, b - a), pl.ds(r0, 8), pl.ds(c0, nc)],
                dst.at[pl.ds(a, b - a), pl.ds(r0, 8), pl.ds(c0, nc)], sems.at[s])
        return Unit(cp(g0, g1 - 1), cp(g1 - 1, g1), (g1 - g0) * 8 * nc * 2, group, s)

    def row_unit(src, dst, group, s, r0, nr):
        def cp(a, b):
            return lambda: pltpu.make_async_copy(
                src.at[pl.ds(r0 + a, b - a)], dst.at[pl.ds(r0 + a, b - a)], sems.at[s])
        return Unit(cp(0, nr - 8), cp(nr - 8, nr), nr * src.shape[-1] * 2, group, s)

    def kv_units(g, p):
        group = ("kv", g)
        if g >= 2 * NSL:
            g, p = g - 2 * NSL, p + 1
        src = k_hbm if g < NSL else v_hbm
        c0 = OFF + (g % NSL) * SC
        slot = g % NS

        def cp(u, a, b):
            return lambda: pltpu.make_async_copy(
                src.at[pl.ds(p * PAIR + u * UR + a, b - a), pl.ds(c0, SC)],
                kv_buf.at[slot, pl.ds(u * UR + a, b - a)], sems.at[slot])
        return [Unit(cp(u, 0, UR - 8), cp(u, UR - 8, UR), KV_UNIT_BYTES, group, slot) for u in range(U)]

    n_wq = (D // WQ_G // 8) * (HQ * DH // SC)
    n_wo = (PAIR // 8) * (len(WO_SPLIT) - 1)
    labels = GroupLabels((-(-(-n_wq // WQ_PER) + -(-n_wo // WO_PER))) % NS)
    x_sem = (labels.first_sem - 1) % NS
    wq_units, wo_units = [], []
    for j in range(D // WQ_G // 8):
        for c in range(HQ * DH // SC):
            grp, s = labels.label("wq", len(wq_units), WQ_PER)
            wq_units.append(view_unit(wq_hbm, wq_v, grp, s, 0, WQ_G, 8 * j, c * SC, SC))
    for j in range(PAIR // 8):
        for k in range(len(WO_SPLIT) - 1):
            grp, s = labels.label("wo", len(wo_units), WO_PER)
            wo_units.append(view_unit(wo_hbm, wo_v, grp, s, WO_SPLIT[k], WO_SPLIT[k + 1], 8 * j, 0, D))
    labels = GroupLabels(0)
    w1_units, w3_units, w2_pieces = [], [], []
    for units, src, dst, tag in ((w1_units, w1_hbm, w1_v, "w1"), (w3_units, w3_hbm, w3_v, "w3")):
        for j in range(D // W13_G // 8):
            for c in range(F // SC):
                grp, s = labels.label(tag, len(units), W13_PER)
                units.append(view_unit(src, dst, grp, s, 0, W13_G, 8 * j, c * SC, SC))
    lo = 0
    for i, (rows, ur) in enumerate(W2_PIECES):
        units = []
        for j in range(rows // ur):
            grp, s = labels.label(("w2", i), j, W2_PER)
            units.append(row_unit(w2_hbm, w2_v, grp, s, lo + ur * j, ur))
        w2_pieces.append((lo, lo + rows, units))
        lo += rows
    assert lo == F and W2_PIECES[-1][0] == 128

    x_cp = pltpu.make_async_copy(x_hbm, x_v, sems.at[x_sem])
    first_kv = [u for g in range(NS - 1) for u in kv_units(g, 0)][:NLO]
    pro = Pump(wq_units + wo_units + first_kv)
    x_cp.start()
    pro.left["x"] = 1
    pro.claim(x_sem, "x")
    pro.fill()
    pro.wait_units(2)
    x_cp.wait()
    pro.left["x"] = 0
    x8 = jnp.broadcast_to(x_v[...].astype(jnp.float32), (8, D))
    xn = _layernorm(x8).astype(jnp.bfloat16)
    pro.wait_units(len(wq_units) - 2)
    pro.landed(wq_units)

    row = jax.lax.broadcasted_iota(jnp.int32, (8, PAIR), 0)
    col = jax.lax.broadcasted_iota(jnp.int32, (8, PAIR), 1)
    diag = ((row == 0) & (col < DH)) | ((row == 1) & (col >= DH))

    def q_piece(j):
        def f():
            w = wq_v[:, :, j * PAIR:(j + 1) * PAIR].reshape(D, PAIR)
            qp = jnp.dot(xn, w, preferred_element_type=jnp.float32)
            q_blk[j] = jnp.where(diag, qp, 0.0).astype(jnp.bfloat16)
        return f

    pro.wait_units(len(wo_units), [q_piece(j) for j in range(NPAIR)])
    pro.landed(wo_units)
    n_pro = len(wq_units) + len(wo_units)
    assert (pro.n_lo, pro.n_hi, pro.n_waited) == (n_pro + NLO, n_pro + MHI, n_pro)

    scale = DH ** -0.5

    def qk_piece(p, i, t):
        s = jnp.dot(q_blk[p], kv_buf[i % NS], preferred_element_type=jnp.float32) * scale
        s_ref[:, i * SC:(i + 1) * SC] = s
        for c in range(SC // 128):
            sc = s[:, c * 128:(c + 1) * 128]
            t["mx"] = sc if "mx" not in t else jnp.maximum(t["mx"], sc)

    def pv_piece(i, t):
        if i == 0:
            t["m"] = jnp.max(t["mx"], axis=-1, keepdims=True)
        e = jnp.exp(s_ref[:, i * SC:(i + 1) * SC] - t["m"])
        for c in range(SC // 128):
            ec = e[:, c * 128:(c + 1) * 128]
            t["l"] = ec if "l" not in t else t["l"] + ec
        o = jax.lax.dot_general(e.astype(jnp.bfloat16), kv_buf[(NSL + i) % NS], NT,
                                preferred_element_type=jnp.float32)
        t["o"] = o if "o" not in t else t["o"] + o

    def slice_compute(p, g, t):
        if g < NSL:
            qk_piece(p, g, t)
        else:
            pv_piece(g - NSL, t)

    def finalize(p, t, acc):
        l = jnp.sum(t["l"], axis=-1, keepdims=True)
        o = jnp.where(diag, t["o"] / l, 0.0).astype(jnp.bfloat16)
        return acc + jnp.dot(o, wo_v[p], preferred_element_type=jnp.float32)

    def pair_body(p, acc):
        t = {}
        for g in range(2 * NSL):
            cur = kv_units(g, p)
            for u in range(U):
                cur[u].hi().wait()
                cur[u].lo().wait()
                il, ih = g * U + u + NLO, g * U + u + MHI
                kv_units(il // U, p)[il % U].lo().start(priority=1)
                kv_units(ih // U, p)[ih % U].hi().start(priority=0)
            slice_compute(p, g, t)
        return finalize(p, t, acc)

    acc = jax.lax.fori_loop(0, NPAIR - 1, pair_body, jnp.zeros((8, D), jnp.float32))

    last = NPAIR - 1
    kv_last = [kv_units(g, last) for g in range(2 * NSL)]
    epi = Pump([u for us in kv_last for u in us] + w1_units + w3_units
               + [u for piece in w2_pieces for u in piece[2]], lo_started=NLO, hi_started=MHI)
    t = {}
    for g in range(2 * NSL):
        epi.wait_units(U)
        epi.landed(kv_last[g])
        slice_compute(last, g, t)
    acc = finalize(last, t, acc)

    attn = jnp.sum(acc, axis=0, keepdims=True)
    h = x8 + jnp.broadcast_to(attn, (8, D))
    hn = _layernorm(h).astype(jnp.bfloat16)
    gc = F // NG
    gate, mid = [None] * NG, [None] * NG

    def gate_piece(i):
        def f():
            w = w1_v[:, :, i * gc:(i + 1) * gc].reshape(D, gc)
            gate[i] = jnp.dot(hn, w, preferred_element_type=jnp.float32)
        return f

    def up_piece(i):
        def f():
            w = w3_v[:, :, i * gc:(i + 1) * gc].reshape(D, gc)
            up = jnp.dot(hn, w, preferred_element_type=jnp.float32)
            mid[i] = (gate[i] * jax.nn.sigmoid(gate[i]) * up).astype(jnp.bfloat16)
        return f

    epi.wait_units(len(w1_units))
    epi.landed(w1_units)
    epi.wait_units(len(w3_units), [gate_piece(i) for i in range(NG)])
    epi.landed(w3_units)
    out = h
    for i, (lo, hi, units) in enumerate(w2_pieces):
        epi.wait_units(len(units), [up_piece(c) for c in range(NG)] if i == 0 else ())
        epi.landed(units)
        if i == 0:
            midc = jnp.concatenate(mid, axis=1)
            mid_t = jnp.broadcast_to(midc[0:1, F - 128:].astype(jnp.float32), (128, 128)).T
        if hi < F:
            out = out + jnp.dot(midc[:, lo:hi], w2_v[lo:hi, :], preferred_element_type=jnp.float32)
        else:
            parts = []
            for c in range(D // 128):
                w = w2_v[lo:hi, c * 128:(c + 1) * 128].astype(jnp.float32)
                parts.append(jnp.sum((w * mid_t).reshape(128 // 8, 8, 128), axis=0))
            out = out[0:1, :] + jnp.sum(jnp.concatenate(parts, axis=1), axis=0, keepdims=True)
    assert epi.n_waited == len(epi.units)
    o_ref[...] = out.astype(o_ref.dtype)


@jax.jit
def pallas_sequential_preLN__sliding_block_cached__glu_gated_swiglu__decode_kernel(
    A_x: jax.Array,
    A_k_cache: jax.Array,
    A_v_cache: jax.Array,
    A_wq: jax.Array,
    A_wo: jax.Array,
    B_x: jax.Array,
    B_w1: jax.Array,
    B_w3: jax.Array,
    B_w2: jax.Array,
):
    del B_x
    assert A_x.shape == (1, 1, D) and A_k_cache.shape == A_v_cache.shape == (1, HQ, SK, DH)
    hbm = pl.BlockSpec(memory_space=pltpu.HBM)
    out = pl.pallas_call(
        _kernel,
        out_shape=jax.ShapeDtypeStruct((1, D), A_x.dtype),
        in_specs=[hbm] * 8,
        out_specs=pl.BlockSpec(memory_space=pltpu.VMEM),
        scratch_shapes=[
            pltpu.VMEM((1, D), jnp.bfloat16),
            pltpu.VMEM((WQ_G, D // WQ_G, HQ * DH), jnp.bfloat16),
            pltpu.VMEM((NPAIR, PAIR, D), jnp.bfloat16),
            pltpu.VMEM((W13_G, D // W13_G, F), jnp.bfloat16),
            pltpu.VMEM((W13_G, D // W13_G, F), jnp.bfloat16),
            pltpu.VMEM((F, D), jnp.bfloat16),
            pltpu.VMEM((NS, PAIR, SC), jnp.bfloat16),
            pltpu.VMEM((NPAIR, 8, PAIR), jnp.bfloat16),
            pltpu.VMEM((8, WIN), jnp.float32),
            pltpu.SemaphoreType.DMA((NS,)),
        ],
        compiler_params=pltpu.CompilerParams(vmem_limit_bytes=64 * 1024 * 1024),
        name="fused_decode_block",
    )(
        A_x.reshape(1, D),
        jnp.transpose(A_k_cache, (0, 1, 3, 2)).reshape(HQ * DH, SK),
        jnp.transpose(A_v_cache, (0, 1, 3, 2)).reshape(HQ * DH, SK),
        A_wq.reshape(WQ_G, D // WQ_G, HQ * DH),
        A_wo.reshape(NPAIR, PAIR, D),
        B_w1.reshape(W13_G, D // W13_G, F),
        B_w3.reshape(W13_G, D // W13_G, F),
        B_w2,
    )
    return out.reshape(1, 1, D)
```

```python
import jax
import jax.numpy as jnp
from jax.experimental import pallas as pl
from jax.experimental.pallas import tpu as pltpu

D = 640
HQ = 32
DH = 192
SK = 32768
WIN = min(4096, max(256, SK // 4))
F = 1536
EPS = 1e-5

PAIR = 2 * DH
NPAIR = HQ // 2
OFF = SK - WIN
SC = 512
NSL = WIN // SC
NH = 4 * NSL
NS = 4
HU = 4
U = 2 * HU
UR = DH // HU
KV_UNIT_BYTES = UR * SC * 2
NLO = 24
MHI = 16
IN_FLIGHT = NLO * KV_UNIT_BYTES
assert U <= MHI <= NLO <= (NS - 1) * U

WQ_G = 8
WO_SPLIT = (0, 6, 11, 16)
W13_G = 4
W2_PIECES = ((768, 48), (384, 48), (256, 32), (128, 32))
WQ_PER, WO_PER, W13_PER, W2_PER = 8, 12, 12, 8
NG = 6
NT = (((1,), (1,)), ((), ()))


def _layernorm(x):
    m = jnp.mean(x, axis=-1, keepdims=True)
    xc = x - m
    v = jnp.mean(xc * xc, axis=-1, keepdims=True)
    return xc / jnp.sqrt(v + EPS)


class Unit:
    def __init__(self, lo, hi, nbytes, group, sem_id):
        self.lo, self.hi, self.nbytes = lo, hi, nbytes
        self.group, self.sem_id = group, sem_id


class Pump:
    def __init__(self, units, lo_started=0, hi_started=0):
        self.units = units
        self.n_lo, self.n_hi, self.n_waited = lo_started, hi_started, 0
        self.inflight = sum(u.nbytes for u in units[:lo_started])
        self.left, self.last = {}, {}
        for i, u in enumerate(units):
            self.left[u.group] = self.left.get(u.group, 0) + 1
            self.last[u.group] = i
        self.owner = {}
        for u in units[:lo_started]:
            self.claim(u.sem_id, u.group)

    def claim(self, sem_id, group):
        prev = self.owner.get(sem_id)
        assert prev is None or prev == group or self.left[prev] == 0, ("semaphore in use", sem_id, prev, group)
        self.owner[sem_id] = group

    def fill(self):
        while self.n_lo < len(self.units) and self.inflight + self.units[self.n_lo].nbytes <= IN_FLIGHT:
            u = self.units[self.n_lo]
            self.claim(u.sem_id, u.group)
            u.lo().start(priority=1)
            self.inflight += u.nbytes
            self.n_lo += 1
        while self.n_hi < min(self.n_lo, self.n_waited + MHI):
            self.units[self.n_hi].hi().start(priority=0)
            self.n_hi += 1

    def step(self):
        u = self.units[self.n_waited]
        assert self.last[u.group] < self.n_hi <= self.n_lo, ("group not fully started", u.group)
        u.hi().wait()
        u.lo().wait()
        self.left[u.group] -= 1
        self.inflight -= u.nbytes
        self.n_waited += 1
        self.fill()

    def wait_units(self, n, pieces=()):
        done = 0
        for i in range(n):
            self.step()
            while done < ((i + 1) * len(pieces)) // n:
                pieces[done]()
                done += 1

    def landed(self, units):
        assert all(self.left[u.group] == 0 for u in units)


class GroupLabels:
    def __init__(self, first_sem):
        self.count, self.first_sem = -1, first_sem

    def label(self, tag, i, per):
        if i % per == 0:
            self.count += 1
        return (tag, i // per), (self.first_sem + self.count) % NS


def _kernel(x_hbm, k_hbm, v_hbm, wq_hbm, wo_hbm, w1_hbm, w3_hbm, w2_hbm,
            o_ref,
            x_v, wq_v, wo_v, w1_v, w3_v, w2_v, kv_buf, q_ref, s_ref, sems):

    def view_unit(src, dst, group, s, g0, g1, r0, c0, nc):
        def cp(a, b):
            return lambda: pltpu.make_async_copy(
                src.at[pl.ds(a, b - a), pl.ds(r0, 8), pl.ds(c0, nc)],
                dst.at[pl.ds(a, b - a), pl.ds(r0, 8), pl.ds(c0, nc)], sems.at[s])
        return Unit(cp(g0, g1 - 1), cp(g1 - 1, g1), (g1 - g0) * 8 * nc * 2, group, s)

    def row_unit(src, dst, group, s, r0, nr):
        def cp(a, b):
            return lambda: pltpu.make_async_copy(
                src.at[pl.ds(r0 + a, b - a)], dst.at[pl.ds(r0 + a, b - a)], sems.at[s])
        return Unit(cp(0, nr - 8), cp(nr - 8, nr), nr * src.shape[-1] * 2, group, s)

    def kv_units(g, p):
        group = ("kv", g // 2)
        if g >= NH:
            g, p = g - NH, p + 1
        head, is_v, c = g // (2 * NSL), (g // NSL) % 2, g % NSL
        src = v_hbm if is_v else k_hbm
        slot, sem = g % (2 * NS), (g // 2) % NS

        def cp(u, a, b):
            return lambda: pltpu.make_async_copy(
                src.at[pl.ds(p * PAIR + head * DH + u * UR + a, b - a), pl.ds(OFF + c * SC, SC)],
                kv_buf.at[slot, pl.ds(u * UR + a, b - a)], sems.at[sem])
        return [Unit(cp(u, 0, UR - 8), cp(u, UR - 8, UR), KV_UNIT_BYTES, group, sem) for u in range(HU)]

    def kv_group(k, p):
        return kv_units(2 * k, p) + kv_units(2 * k + 1, p)

    n_wq = (D // WQ_G // 8) * (HQ * DH // SC)
    n_wo = (PAIR // 8) * (len(WO_SPLIT) - 1)
    labels = GroupLabels((-(-(-n_wq // WQ_PER) + -(-n_wo // WO_PER))) % NS)
    x_sem = (labels.first_sem - 1) % NS
    wq_units, wo_units = [], []
    for j in range(D // WQ_G // 8):
        for c in range(HQ * DH // SC):
            grp, s = labels.label("wq", len(wq_units), WQ_PER)
            wq_units.append(view_unit(wq_hbm, wq_v, grp, s, 0, WQ_G, 8 * j, c * SC, SC))
    for j in range(PAIR // 8):
        for k in range(len(WO_SPLIT) - 1):
            grp, s = labels.label("wo", len(wo_units), WO_PER)
            wo_units.append(view_unit(wo_hbm, wo_v, grp, s, WO_SPLIT[k], WO_SPLIT[k + 1], 8 * j, 0, D))
    labels = GroupLabels(0)
    w1_units, w3_units, w2_pieces = [], [], []
    for units, src, dst, tag in ((w1_units, w1_hbm, w1_v, "w1"), (w3_units, w3_hbm, w3_v, "w3")):
        for j in range(D // W13_G // 8):
            for c in range(F // SC):
                grp, s = labels.label(tag, len(units), W13_PER)
                units.append(view_unit(src, dst, grp, s, 0, W13_G, 8 * j, c * SC, SC))
    lo = 0
    for i, (rows, ur) in enumerate(W2_PIECES):
        units = []
        for j in range(rows // ur):
            grp, s = labels.label(("w2", i), j, W2_PER)
            units.append(row_unit(w2_hbm, w2_v, grp, s, lo + ur * j, ur))
        w2_pieces.append((lo, lo + rows, units))
        lo += rows
    assert lo == F and W2_PIECES[-1][0] == 128

    x_cp = pltpu.make_async_copy(x_hbm, x_v, sems.at[x_sem])
    first_kv = [u for k in range(NS - 1) for u in kv_group(k, 0)][:NLO]
    pro = Pump(wq_units + wo_units + first_kv)
    x_cp.start()
    pro.left["x"] = 1
    pro.claim(x_sem, "x")
    pro.fill()
    pro.wait_units(2)
    x_cp.wait()
    pro.left["x"] = 0
    x8 = jnp.broadcast_to(x_v[...].astype(jnp.float32), (8, D))
    xn = _layernorm(x8).astype(jnp.bfloat16)
    pro.wait_units(len(wq_units) - 2)
    pro.landed(wq_units)

    def q_piece(j):
        def f():
            w = wq_v[:, :, j * PAIR:(j + 1) * PAIR].reshape(D, PAIR)
            q = jnp.dot(xn, w, preferred_element_type=jnp.float32).astype(jnp.bfloat16)
            q_ref[2 * j] = q[:, :DH]
            q_ref[2 * j + 1] = q[:, DH:]
        return f

    pro.wait_units(len(wo_units), [q_piece(j) for j in range(NPAIR)])
    pro.landed(wo_units)
    n_pro = len(wq_units) + len(wo_units)
    assert (pro.n_lo, pro.n_hi, pro.n_waited) == (n_pro + NLO, n_pro + MHI, n_pro)

    scale = DH ** -0.5

    def qk_piece(head, g, t):
        i = g % NSL
        s = jnp.dot(q_ref[head], kv_buf[g % (2 * NS)], preferred_element_type=jnp.float32) * scale
        s_ref[:, i * SC:(i + 1) * SC] = s
        for c in range(SC // 128):
            sc = s[:, c * 128:(c + 1) * 128]
            t["mx"] = sc if "mx" not in t else jnp.maximum(t["mx"], sc)

    def pv_piece(g, t):
        i = g % NSL
        if i == 0:
            t["m"] = jnp.max(t["mx"], axis=-1, keepdims=True)
        e = jnp.exp(s_ref[:, i * SC:(i + 1) * SC] - t["m"])
        for c in range(SC // 128):
            ec = e[:, c * 128:(c + 1) * 128]
            t["l"] = ec if "l" not in t else t["l"] + ec
        o = jax.lax.dot_general(e.astype(jnp.bfloat16), kv_buf[g % (2 * NS)], NT,
                                preferred_element_type=jnp.float32)
        t["o"] = o if "o" not in t else t["o"] + o

    def group_compute(p, k, t, acc):
        for g in (2 * k, 2 * k + 1):
            head, is_v = g // (2 * NSL), (g // NSL) % 2
            if is_v:
                pv_piece(g, t)
            else:
                qk_piece(2 * p + head, g, t)
            if g % (2 * NSL) == 2 * NSL - 1:
                o = (t["o"] / jnp.sum(t["l"], axis=-1, keepdims=True)).astype(jnp.bfloat16)
                acc = acc + jnp.dot(o, wo_v[p, head * DH:(head + 1) * DH, :],
                                    preferred_element_type=jnp.float32)
                t.clear()
        return acc

    def pair_body(p, acc):
        t = {}
        for k in range(NH // 2):
            cur = kv_group(k, p)
            for u in range(U):
                cur[u].hi().wait()
                cur[u].lo().wait()
                il, ih = k * U + u + NLO, k * U + u + MHI
                kv_units(il // HU, p)[il % HU].lo().start(priority=1)
                kv_units(ih // HU, p)[ih % HU].hi().start(priority=0)
            acc = group_compute(p, k, t, acc)
        return acc

    acc = jax.lax.fori_loop(0, NPAIR - 1, pair_body, jnp.zeros((8, D), jnp.float32))

    last = NPAIR - 1
    kv_last = [kv_group(k, last) for k in range(NH // 2)]
    epi = Pump([u for us in kv_last for u in us] + w1_units + w3_units
               + [u for piece in w2_pieces for u in piece[2]], lo_started=NLO, hi_started=MHI)
    t = {}
    for k in range(NH // 2):
        epi.wait_units(U)
        epi.landed(kv_last[k])
        acc = group_compute(last, k, t, acc)

    h = x8 + acc
    hn = _layernorm(h).astype(jnp.bfloat16)
    gc = F // NG
    gate, mid = [None] * NG, [None] * NG

    def gate_piece(i):
        def f():
            w = w1_v[:, :, i * gc:(i + 1) * gc].reshape(D, gc)
            gate[i] = jnp.dot(hn, w, preferred_element_type=jnp.float32)
        return f

    def up_piece(i):
        def f():
            w = w3_v[:, :, i * gc:(i + 1) * gc].reshape(D, gc)
            up = jnp.dot(hn, w, preferred_element_type=jnp.float32)
            mid[i] = (gate[i] * jax.nn.sigmoid(gate[i]) * up).astype(jnp.bfloat16)
        return f

    epi.wait_units(len(w1_units))
    epi.landed(w1_units)
    epi.wait_units(len(w3_units), [gate_piece(i) for i in range(NG)])
    epi.landed(w3_units)
    out = h
    for i, (lo, hi, units) in enumerate(w2_pieces):
        epi.wait_units(len(units), [up_piece(c) for c in range(NG)] if i == 0 else ())
        epi.landed(units)
        if i == 0:
            midc = jnp.concatenate(mid, axis=1)
            mid_t = jnp.broadcast_to(midc[0:1, F - 128:].astype(jnp.float32), (128, 128)).T
        if hi < F:
            out = out + jnp.dot(midc[:, lo:hi], w2_v[lo:hi, :], preferred_element_type=jnp.float32)
        else:
            parts = []
            for c in range(D // 128):
                w = w2_v[lo:hi, c * 128:(c + 1) * 128].astype(jnp.float32)
                parts.append(jnp.sum((w * mid_t).reshape(128 // 8, 8, 128), axis=0))
            out = out[0:1, :] + jnp.sum(jnp.concatenate(parts, axis=1), axis=0, keepdims=True)
    assert epi.n_waited == len(epi.units)
    o_ref[...] = out.astype(o_ref.dtype)


@jax.jit
def pallas_sequential_preLN__sliding_block_cached__glu_gated_swiglu__decode_kernel(
    A_x: jax.Array,
    A_k_cache: jax.Array,
    A_v_cache: jax.Array,
    A_wq: jax.Array,
    A_wo: jax.Array,
    B_x: jax.Array,
    B_w1: jax.Array,
    B_w3: jax.Array,
    B_w2: jax.Array,
):
    del B_x
    assert A_x.shape == (1, 1, D) and A_k_cache.shape == A_v_cache.shape == (1, HQ, SK, DH)
    hbm = pl.BlockSpec(memory_space=pltpu.HBM)
    out = pl.pallas_call(
        _kernel,
        out_shape=jax.ShapeDtypeStruct((1, D), A_x.dtype),
        in_specs=[hbm] * 8,
        out_specs=pl.BlockSpec(memory_space=pltpu.VMEM),
        scratch_shapes=[
            pltpu.VMEM((1, D), jnp.bfloat16),
            pltpu.VMEM((WQ_G, D // WQ_G, HQ * DH), jnp.bfloat16),
            pltpu.VMEM((NPAIR, PAIR, D), jnp.bfloat16),
            pltpu.VMEM((W13_G, D // W13_G, F), jnp.bfloat16),
            pltpu.VMEM((W13_G, D // W13_G, F), jnp.bfloat16),
            pltpu.VMEM((F, D), jnp.bfloat16),
            pltpu.VMEM((2 * NS, DH, SC), jnp.bfloat16),
            pltpu.VMEM((HQ, 8, DH), jnp.bfloat16),
            pltpu.VMEM((8, WIN), jnp.float32),
            pltpu.SemaphoreType.DMA((NS,)),
        ],
        compiler_params=pltpu.CompilerParams(vmem_limit_bytes=64 * 1024 * 1024),
        name="fused_decode_block",
    )(
        A_x.reshape(1, D),
        jnp.transpose(A_k_cache, (0, 1, 3, 2)).reshape(HQ * DH, SK),
        jnp.transpose(A_v_cache, (0, 1, 3, 2)).reshape(HQ * DH, SK),
        A_wq.reshape(WQ_G, D // WQ_G, HQ * DH),
        A_wo.reshape(NPAIR, PAIR, D),
        B_w1.reshape(W13_G, D // W13_G, F),
        B_w3.reshape(W13_G, D // W13_G, F),
        B_w2,
    )
    return out.reshape(1, 1, D)
```
